```python
import os as _os
_os.environ.setdefault("JAX_PLATFORMS", "cpu")
import jax
import jax.numpy as jnp

def _softmax(x, axis=-1):
    return jax.nn.softmax(x, axis=axis)
def _gelu(x):
    return jax.nn.gelu(x, approximate=True)
def _silu(x):
    return jax.nn.silu(x)
def _sigmoid(x):
    return jax.nn.sigmoid(x)
def _layernorm(x, axis=-1, eps=1e-5):
    m = jnp.mean(x, axis=axis, keepdims=True)
    v = jnp.var(x, axis=axis, keepdims=True)
    return (x - m) / jnp.sqrt(v + eps)
def _scatter_add(tgt, idx, src, axis=0):
    return tgt.at[idx].add(src)
def _segment_sum(src, seg, n):
    return jax.ops.segment_sum(src, seg, n)
class _Rng:
    def __init__(self, key):
        self._k = key
    def _next(self):
        self._k, sub = jax.random.split(self._k)
        return sub
    def normal(self, shape):
        return jax.random.normal(self._next(), shape, dtype=jnp.bfloat16)
    def randint(self, lo, hi, shape):
        return jax.random.randint(self._next(), shape, lo, hi, dtype=jnp.int32)
    def uniform(self, shape, lo=0.0, hi=1.0):
        return jax.random.uniform(self._next(), shape, jnp.bfloat16, lo, hi)
    def permutation(self, n):
        return jax.random.permutation(self._next(), n)


kernel_name = 'sequential_preLN__softmax_full_mha__glu_gated_swiglu__prompt'

def setup_inputs():
    _rng = _Rng(jax.random.key(int.from_bytes(__import__("os").urandom(4), "little")))
    _w = (lambda a: (lambda t: t.astype(jnp.bfloat16) if jnp.issubdtype(t.dtype, jnp.floating) else t)(jnp.asarray(a)))
    def _A_setup():
        B, S, D = 1, 2048, 640
        return {
            "x": _w((lambda *s: _rng.normal(s) * 0.05)(B, S, D)),
            "wqkv": _w((lambda *s: _rng.normal(s) * 0.05)(D, 3 * D)),
            "wo": _w((lambda *s: _rng.normal(s) * 0.05)(D, D)),
        }
    _A_in = _A_setup()

    def _B_setup():
        B, S, D, F = 1, 2048, 640, 1728
        return {
            "x": _w((lambda *s: _rng.normal(s) * 0.05)(B, S, D)),
            "w1": _w((lambda *s: _rng.normal(s) * 0.05)(D, F) * (2.0 / D) ** 0.5),
            "w3": _w((lambda *s: _rng.normal(s) * 0.05)(D, F) * (2.0 / D) ** 0.5),
            "w2": _w((lambda *s: _rng.normal(s) * 0.05)(F, D) * (2.0 / F) ** 0.5),
        }
    _B_in = _B_setup()

    return {
        "A_x": _A_in["x"],
        "A_wqkv": _A_in["wqkv"],
        "A_wo": _A_in["wo"],
        "B_x": _B_in["x"],
        "B_w1": _B_in["w1"],
        "B_w3": _B_in["w3"],
        "B_w2": _B_in["w2"],
    }

def reference(A_x, A_wqkv, A_wo, B_x, B_w1, B_w3, B_w2):
    def _A_ref(x, wqkv, wo):
        B, S, D = x.shape
        H = 32; Dh = D // H
        qkv = (lambda x, *d: x.transpose(*d))((x @ wqkv).reshape(B, S, 3, H, Dh), 2, 0, 3, 1, 4)
        q, k, v = qkv[0], qkv[1], qkv[2]
        scale = Dh ** -0.5
        scores = jnp.einsum("bhqd,bhkd->bhqk", q, k) * scale
        p = _softmax(scores, axis=-1)
        o = jnp.einsum("bhqk,bhkd->bhqd", p, v)
        return (lambda x, *d: x.transpose(*d))(o, 0, 2, 1, 3).reshape(B, S, D) @ wo

    def _B_ref(x, w1, w3, w2):
        gate = jnp.einsum("bsd,df->bsf", x, w1)
        up = jnp.einsum("bsd,df->bsf", x, w3)
        h = _silu(gate) * up
        out = jnp.einsum("bsf,fd->bsd", h, w2)
        return out

    x = A_x
    h = x + _A_ref(_layernorm(x, axis=-1), A_wqkv, A_wo)
    h2 = h + _B_ref(_layernorm(h, axis=-1), B_w1, B_w3, B_w2)
    return h2
```

```python
import jax
import jax.numpy as jnp
from jax import lax
import jax.experimental.pallas as pl
import jax.experimental.pallas.tpu as pltpu

H = 32
DH = 20
DHP = 32
EPS = 1e-5


def _layernorm_f32(x):
    m = jnp.mean(x, axis=-1, keepdims=True)
    xc = x - m
    v = jnp.mean(xc * xc, axis=-1, keepdims=True)
    return xc * lax.rsqrt(v + EPS)


def _make_kernel(S, D, F, TQ, RC):
    DP = H * DHP
    NG = DP // 128
    HPG = 128 // DHP
    scale = DH ** -0.5

    def kernel(x_ref, wqkv_ref, wo_ref, w1_ref, w3_ref, w2_ref, out_ref,
               qkv_s, kT_s, o_s):
        step = pl.program_id(0)

        @pl.when(step == 0)
        def _():
            def proj(c, carry):
                r = pl.multiple_of(c * RC, RC)
                xc = x_ref[pl.ds(r, RC), :].astype(jnp.float32)
                ln = _layernorm_f32(xc).astype(jnp.bfloat16)
                qkv_c = jnp.dot(ln, wqkv_ref[...],
                                preferred_element_type=jnp.float32)
                qkv_bf = qkv_c.astype(jnp.bfloat16)
                qkv_s[pl.ds(r, RC), :] = qkv_bf
                kT_s[:, pl.ds(r, RC)] = jnp.transpose(
                    qkv_c[:, DP:2 * DP]).astype(jnp.bfloat16)
                return carry
            lax.fori_loop(0, S // RC, proj, 0)

        r0 = pl.multiple_of(step * TQ, TQ)
        lane = lax.broadcasted_iota(jnp.int32, (TQ, 128), 1)

        def group(g, carry):
            off = pl.multiple_of(g * 128, 128)
            qg = qkv_s[pl.ds(r0, TQ), pl.ds(off, 128)]
            kTg = kT_s[pl.ds(off, 128), :]
            vg = qkv_s[:, pl.ds(pl.multiple_of(2 * DP + off, 128), 128)]
            og = jnp.zeros((TQ, 128), jnp.float32)
            for j in range(HPG):
                mwin = (lane >= j * DHP) & (lane < j * DHP + DH)
                qh = jnp.where(mwin, qg, jnp.zeros_like(qg))
                s = jnp.dot(qh, kTg, preferred_element_type=jnp.float32)
                m = jnp.max(s, axis=-1, keepdims=True)
                e = jnp.exp((s - m) * scale)
                den = jnp.sum(e, axis=-1, keepdims=True)
                oh = jnp.dot(e.astype(jnp.bfloat16), vg,
                             preferred_element_type=jnp.float32)
                oh = oh * (1.0 / den)
                og = jnp.where(mwin, oh, og)
            o_s[:, pl.ds(off, 128)] = og.astype(jnp.bfloat16)
            return carry
        lax.fori_loop(0, NG, group, 0)

        attn = jnp.dot(o_s[...], wo_ref[...], preferred_element_type=jnp.float32)
        xb = x_ref[pl.ds(r0, TQ), :].astype(jnp.float32)
        h = xb + attn

        lnh = _layernorm_f32(h).astype(jnp.bfloat16)
        gate = jnp.dot(lnh, w1_ref[...], preferred_element_type=jnp.float32)
        up = jnp.dot(lnh, w3_ref[...], preferred_element_type=jnp.float32)
        act = (gate * jax.nn.sigmoid(gate)) * up
        ffn = jnp.dot(act.astype(jnp.bfloat16), w2_ref[...],
                      preferred_element_type=jnp.float32)
        out_ref[...] = (h + ffn).astype(out_ref.dtype)

    return kernel, DP


@jax.jit
def pallas_sequential_preLN__softmax_full_mha__glu_gated_swiglu__prompt_kernel(
    A_x: jax.Array,
    A_wqkv: jax.Array,
    A_wo: jax.Array,
    B_x: jax.Array,
    B_w1: jax.Array,
    B_w3: jax.Array,
    B_w2: jax.Array,
):
    B, S, D = A_x.shape
    F = B_w1.shape[1]
    assert B == 1
    TQ = 512
    RC = 256

    x2 = A_x.reshape(S, D)
    wqkv_p = jnp.pad(A_wqkv.reshape(D, 3, H, DH),
                     ((0, 0), (0, 0), (0, 0), (0, DHP - DH))).reshape(D, 3 * H * DHP)
    wo_p = jnp.pad(A_wo.reshape(H, DH, D),
                   ((0, 0), (0, DHP - DH), (0, 0))).reshape(H * DHP, D)

    kernel, DP = _make_kernel(S, D, F, TQ, RC)

    full = lambda i: (0, 0)
    out = pl.pallas_call(
        kernel,
        grid=(S // TQ,),
        in_specs=[
            pl.BlockSpec((S, D), full),
            pl.BlockSpec((D, 3 * DP), full),
            pl.BlockSpec((DP, D), full),
            pl.BlockSpec((D, F), full),
            pl.BlockSpec((D, F), full),
            pl.BlockSpec((F, D), full),
        ],
        out_specs=pl.BlockSpec((TQ, D), lambda i: (i, 0)),
        out_shape=jax.ShapeDtypeStruct((S, D), A_x.dtype),
        scratch_shapes=[
            pltpu.VMEM((S, 3 * DP), jnp.bfloat16),
            pltpu.VMEM((DP, S), jnp.bfloat16),
            pltpu.VMEM((TQ, DP), jnp.bfloat16),
        ],
        compiler_params=pltpu.CompilerParams(
            dimension_semantics=("arbitrary",),
            vmem_limit_bytes=112 * 1024 * 1024,
        ),
    )(x2, wqkv_p, wo_p, B_w1, B_w3, B_w2)
    return out.reshape(B, S, D)
```

```python
import jax
import jax.numpy as jnp
from jax import lax
import jax.experimental.pallas as pl
import jax.experimental.pallas.tpu as pltpu

H = 32
DH = 20
HPG = 6
GW = HPG * DH
NG = (H + HPG - 1) // HPG
EPS = 1e-5


def _layernorm_f32(x):
    m = jnp.mean(x, axis=-1, keepdims=True)
    xc = x - m
    v = jnp.mean(xc * xc, axis=-1, keepdims=True)
    return xc * lax.rsqrt(v + EPS)


def _make_kernel(S, D, F, TQ, RC):
    DP = NG * 128
    NFG = H // HPG
    NREM = H - NFG * HPG
    scale = DH ** -0.5

    def kernel(x_ref, wqkv_ref, wo_hbm, w1_hbm, w3_hbm, w2_hbm, out_ref,
               wq_s, wo_s, qkv_s, kT_s, o_s, wo_ref, w1_ref, w3_ref, w2_ref, sems):
        step = pl.program_id(0)

        _srcs = (wo_hbm, w1_hbm, w3_hbm, w2_hbm)
        _dsts = (wo_ref, w1_ref, w3_ref, w2_ref)

        def wcopy(i):
            return pltpu.make_async_copy(_srcs[i], _dsts[i], sems.at[i])

        @pl.when(step == 0)
        def _():
            for i in range(4):
                wcopy(i).start()

        @pl.when(step == 0)
        def _():
            wq_s[...] = jnp.zeros(wq_s.shape, wq_s.dtype)
            wo_s[...] = jnp.zeros(wo_s.shape, wo_s.dtype)
            for g in range(NG):
                nc = min(GW, D - GW * g)
                for t in range(3):
                    wq_s[:, t * DP + 128 * g: t * DP + 128 * g + nc] = (
                        wqkv_ref[:, t * D + GW * g: t * D + GW * g + nc])

            def proj(c, carry):
                r = pl.multiple_of(c * RC, RC)
                xc = x_ref[pl.ds(r, RC), :].astype(jnp.float32)
                ln = _layernorm_f32(xc).astype(jnp.bfloat16)
                qkv_c = jnp.dot(ln, wq_s[...],
                                preferred_element_type=jnp.float32)
                qkv_s[pl.ds(r, RC), :] = qkv_c.astype(jnp.bfloat16)
                kT_s[:, pl.ds(r, RC)] = jnp.transpose(
                    qkv_c[:, DP:2 * DP]).astype(jnp.bfloat16)
                return carry
            lax.fori_loop(0, S // RC, proj, 0)
            wcopy(0).wait()
            for g in range(NG):
                nc = min(GW, D - GW * g)
                wo_s[128 * g: 128 * g + nc, :] = wo_ref[GW * g: GW * g + nc, :]

        r0 = pl.multiple_of(step * TQ, TQ)
        lane = lax.broadcasted_iota(jnp.int32, (TQ, 128), 1)
        vlane = lax.broadcasted_iota(jnp.int32, (S, 128), 1)

        def head_qk(h):
            g = h // HPG
            j = h % HPG
            off = pl.multiple_of(g * 128, 128)
            qg = qkv_s[pl.ds(r0, TQ), pl.ds(off, 128)]
            kTg = kT_s[pl.ds(off, 128), :]
            lo = j * DH
            mwin = (lane >= lo) & (lane < lo + DH)
            qh = jnp.where(mwin, qg * scale, jnp.zeros_like(qg))
            return jnp.dot(qh, kTg, preferred_element_type=jnp.float32)

        def head_pv(h, s):
            g = h // HPG
            j = h % HPG
            off = pl.multiple_of(g * 128, 128)
            voff = pl.multiple_of(off + 2 * DP, 128)
            vg = qkv_s[:, pl.ds(voff, 128)]
            vg1 = jnp.where(vlane == GW, jnp.ones_like(vg), vg)
            lo = j * DH
            mwin = (lane >= lo) & (lane < lo + DH)
            m = jnp.max(s, axis=-1, keepdims=True)
            e = jnp.exp(s - m)
            oh = jnp.dot(e.astype(jnp.bfloat16), vg1,
                         preferred_element_type=jnp.float32)
            den = jnp.sum(jnp.where(lane == GW, oh, 0.0), axis=-1, keepdims=True)
            oh = oh * (1.0 / den)
            og = o_s[:, pl.ds(off, 128)].astype(jnp.float32)
            og = jnp.where(mwin, oh, og)
            o_s[:, pl.ds(off, 128)] = og.astype(jnp.bfloat16)

        o_s[...] = jnp.zeros(o_s.shape, o_s.dtype)
        def head4(i, carry):
            ss = [head_qk(i * 4 + u) for u in range(4)]
            for u in range(4):
                head_pv(i * 4 + u, ss[u])
            return carry
        lax.fori_loop(0, H // 4, head4, 0)

        attn = jnp.dot(o_s[...], wo_s[...], preferred_element_type=jnp.float32)
        xb = x_ref[pl.ds(r0, TQ), :].astype(jnp.float32)
        h = xb + attn

        @pl.when(step == 0)
        def _():
            for i in range(1, 4):
                wcopy(i).wait()

        lnh = _layernorm_f32(h).astype(jnp.bfloat16)
        nt = (((1,), (1,)), ((), ()))
        gate = lax.dot_general(lnh, w1_ref[...], nt, preferred_element_type=jnp.float32)
        up = lax.dot_general(lnh, w3_ref[...], nt, preferred_element_type=jnp.float32)
        act = (gate * jax.nn.sigmoid(gate)) * up
        ffn = jnp.dot(act.astype(jnp.bfloat16), w2_ref[...],
                      preferred_element_type=jnp.float32)
        out_ref[...] = (h + ffn).astype(out_ref.dtype)

    return kernel, DP


@jax.jit
def pallas_sequential_preLN__softmax_full_mha__glu_gated_swiglu__prompt_kernel(
    A_x: jax.Array,
    A_wqkv: jax.Array,
    A_wo: jax.Array,
    B_x: jax.Array,
    B_w1: jax.Array,
    B_w3: jax.Array,
    B_w2: jax.Array,
):
    B, S, D = A_x.shape
    F = B_w1.shape[1]
    assert B == 1
    TQ = 512
    RC = 256

    x2 = A_x.reshape(S, D)
    kernel, DP = _make_kernel(S, D, F, TQ, RC)

    full = lambda i: (0, 0)
    out = pl.pallas_call(
        kernel,
        grid=(S // TQ,),
        in_specs=[
            pl.BlockSpec((S, D), full),
            pl.BlockSpec((D, 3 * D), full),
            pl.BlockSpec(memory_space=pl.ANY),
            pl.BlockSpec(memory_space=pl.ANY),
            pl.BlockSpec(memory_space=pl.ANY),
            pl.BlockSpec(memory_space=pl.ANY),
        ],
        out_specs=pl.BlockSpec((TQ, D), lambda i: (i, 0)),
        out_shape=jax.ShapeDtypeStruct((S, D), A_x.dtype),
        scratch_shapes=[
            pltpu.VMEM((D, 3 * DP), jnp.bfloat16),
            pltpu.VMEM((DP, D), jnp.bfloat16),
            pltpu.VMEM((S, 3 * DP), jnp.bfloat16),
            pltpu.VMEM((DP, S), jnp.bfloat16),
            pltpu.VMEM((TQ, DP), jnp.bfloat16),
            pltpu.VMEM((D, D), jnp.bfloat16),
            pltpu.VMEM((F, D), jnp.bfloat16),
            pltpu.VMEM((F, D), jnp.bfloat16),
            pltpu.VMEM((F, D), jnp.bfloat16),
            pltpu.SemaphoreType.DMA((4,)),
        ],
        compiler_params=pltpu.CompilerParams(
            dimension_semantics=("arbitrary",),
            vmem_limit_bytes=112 * 1024 * 1024,
        ),
    )(x2, A_wqkv, A_wo, B_w1.T, B_w3.T, B_w2)
    return out.reshape(B, S, D)
```
